```python
import jax
import jax.numpy as jnp

def _softmax(x, axis=-1):
    return jax.nn.softmax(x, axis=axis)

def _gelu(x):
    return jax.nn.gelu(x, approximate=True)

def _silu(x):
    return jax.nn.silu(x)

def _sigmoid(x):
    return jax.nn.sigmoid(x)

def _layernorm(x, axis=-1, eps=1e-05):
    m = jnp.mean(x, axis=axis, keepdims=True)
    v = jnp.var(x, axis=axis, keepdims=True)
    return (x - m) / jnp.sqrt(v + eps)

def _scatter_add(tgt, idx, src, axis=0):
    return tgt.at[idx].add(src)

def _segment_sum(src, seg, n):
    return jax.ops.segment_sum(src, seg, n)

class _Rng:

    def __init__(self, key):
        self._k = key

    def _next(self):
        self._k, sub = jax.random.split(self._k)
        return sub

    def normal(self, shape):
        return jax.random.normal(self._next(), shape, dtype=jnp.bfloat16)

    def randint(self, lo, hi, shape):
        return jax.random.randint(self._next(), shape, lo, hi, dtype=jnp.int32)

    def uniform(self, shape, lo=0.0, hi=1.0):
        return jax.random.uniform(self._next(), shape, jnp.bfloat16, lo, hi)

    def permutation(self, n):
        return jax.random.permutation(self._next(), n)
kernel_name = 'adaLN_cond__sliding_block_cached__dense_activation_gelu__decode'

def setup_inputs():
    _rng = _Rng(jax.random.key(int.from_bytes(__import__("os").urandom(4), "little")))
    _w = lambda a: (lambda t: t.astype(jnp.bfloat16) if jnp.issubdtype(t.dtype, jnp.floating) else t)(jnp.asarray(a))

    def _A_setup():
        B, Sq, D = (4, 1, 640)
        Hq, Hkv, Sk, Dh = (32, 32, 8192, 128)
        assert Hq % Hkv == 0, (Hq, Hkv)
        return {'x': _w((lambda *s: _rng.normal(s) * 0.05)(B, Sq, D)), 'k_cache': _w((lambda *s: _rng.normal(s) * 0.05)(B, Hkv, Sk, Dh)), 'v_cache': _w((lambda *s: _rng.normal(s) * 0.05)(B, Hkv, Sk, Dh)), 'wq': _w((lambda *s: _rng.normal(s) * 0.05)(D, Hq * Dh) * D ** (-0.5)), 'wo': _w((lambda *s: _rng.normal(s) * 0.05)(Hq * Dh, D) * (Hq * Dh) ** (-0.5))}
    _A_in = _A_setup()

    def _B_setup():
        B, S, D, F = (4, 1, 640, 1728)
        return {'x': _w((lambda *s: _rng.normal(s) * 0.05)(B, S, D)), 'w1': _w((lambda *s: _rng.normal(s) * 0.05)(D, F) * D ** (-0.5)), 'b1': _w((lambda *s: _rng.normal(s) * 0.05)(F) * 0.01), 'w2': _w((lambda *s: _rng.normal(s) * 0.05)(F, D) * F ** (-0.5)), 'b2': _w((lambda *s: _rng.normal(s) * 0.05)(D) * 0.01)}
    _B_in = _B_setup()
    return {'A_x': _A_in['x'], 'A_k_cache': _A_in['k_cache'], 'A_v_cache': _A_in['v_cache'], 'A_wq': _A_in['wq'], 'A_wo': _A_in['wo'], 'B_x': _B_in['x'], 'B_w1': _B_in['w1'], 'B_b1': _B_in['b1'], 'B_w2': _B_in['w2'], 'B_b2': _B_in['b2'], 'c': _w((lambda *s: _rng.normal(s) * 0.05)(4, 640)), 'w_mod': _w((lambda *s: _rng.normal(s) * 0.05)(640, 6 * 640) * 640 ** (-0.5))}

def reference(A_x, A_k_cache, A_v_cache, A_wq, A_wo, B_x, B_w1, B_b1, B_w2, B_b2, c, w_mod):

    def _A_ref(x, k_cache, v_cache, wq, wo):
        B, Sq, D = x.shape
        Hq, Dh = (32, 128)
        Hkv, Sk = (k_cache.shape[1], k_cache.shape[2])
        W = min(4096, max(256, Sk // 4))
        rep = Hq // Hkv
        q = (lambda x, *d: x.transpose(*d))((x @ wq).reshape(B, Sq, Hq, Dh), 0, 2, 1, 3)
        k = jnp.repeat(k_cache[:, :, Sk - W:, :], rep, axis=1)
        v = jnp.repeat(v_cache[:, :, Sk - W:, :], rep, axis=1)
        scores = jnp.einsum('bhqd,bhkd->bhqk', q, k) * Dh ** (-0.5)
        p = _softmax(scores, axis=-1)
        o = jnp.einsum('bhqk,bhkd->bhqd', p, v)
        return (lambda x, *d: x.transpose(*d))(o, 0, 2, 1, 3).reshape(B, Sq, Hq * Dh) @ wo

    def _B_ref(x, w1, b1, w2, b2):
        h = jnp.einsum('bsd,df->bsf', x, w1) + b1
        h = _gelu(h)
        return jnp.einsum('bsf,fd->bsd', h, w2) + b2
    x = A_x
    mod = (_silu(c) @ w_mod).reshape(c.shape[0], 6, 1, -1)
    sa, ca, ga, sb, cb, gb = (mod[:, 0].copy(), mod[:, 1].copy(), mod[:, 2].copy(), mod[:, 3].copy(), mod[:, 4].copy(), mod[:, 5].copy())
    h = _layernorm(x, axis=-1) * (1 + ca) + sa
    x = x + ga * _A_ref(h, A_k_cache, A_v_cache, A_wq, A_wo)
    h = _layernorm(x, axis=-1) * (1 + cb) + sb
    x = x + gb * _B_ref(h, B_w1, B_b1, B_w2, B_b2)
    return x
```

```python
import functools
import math

import jax
import jax.numpy as jnp
from jax import lax
import jax.experimental.pallas as pl
import jax.experimental.pallas.tpu as pltpu

F32 = jnp.float32
BF16 = jnp.bfloat16


def _dot(a, b):
    return lax.dot_general(a, b, (((1,), (0,)), ((), ())), preferred_element_type=F32)


def _dot_t(a, b):
    return lax.dot_general(a, b, (((1,), (1,)), ((), ())), preferred_element_type=F32)


def _layernorm(x):
    m = jnp.mean(x, axis=-1, keepdims=True)
    d = x - m
    v = jnp.mean(d * d, axis=-1, keepdims=True)
    return d / jnp.sqrt(v + 1e-05)


def _gelu(x):
    k = math.sqrt(2.0 / math.pi)
    return 0.5 * x * (1.0 + jnp.tanh(k * (x + 0.044715 * (x * x * x))))


def make(NS=16, A=128, DEPTH=3, CT=256, FR=64):
    def kern(x_hbm, c_hbm, b1_hbm, b2_hbm, wmod_hbm, wq_hbm, wo_hbm, w1t_hbm, w2_hbm,
             k_hbm, v_hbm, o_ref,
             x_v, c_v, b1_v, b2_v, wmod_v, wq_v, wo_v, w1t_v, w2_v, kb, vb,
             mod_v, h_v, q_v, oh_v, acc_v, sem_s, sem_w, sem_kv, sem_f):
        B, D = x_hbm.shape
        _, H, SK, DH = k_hbm.shape
        W = kb.shape[1]
        F = w2_hbm.shape[0]
        R = DEPTH + 1
        N = B * H
        row0 = SK - W

        def cp(src, dst, sem, prio):
            pltpu.make_async_copy(src, dst, sem).start(priority=prio)

        def wait(buf, sem):
            pltpu.make_async_copy(buf, buf, sem).wait()

        def ds(i, n):
            return pl.ds(pl.multiple_of(i * n, n), n)

        def wmod_step(i, _):
            for j in range(3):
                for p in range(2):
                    r = ds(i + p * (D // 32), 16)
                    cs = pl.ds(j * 2 * D, 2 * D)
                    cp(wmod_hbm.at[r, cs], wmod_v.at[r, cs], sem_w.at[0], p)

        def wq_step(i, _):
            for j in range(4):
                for p in range(2):
                    r = ds(i + p * (D // 32), 16)
                    cs = pl.ds(j * 1024, 1024)
                    cp(wq_hbm.at[r, cs], wq_v.at[r, cs], sem_w.at[1], p)

        def wo_step(i):
            for p in range(2):
                r = ds(i + p * 64, 32)
                cp(wo_hbm.at[r], wo_v.at[r], sem_w.at[2], p)

        def kv_step(n, slot, s):
            h, b = n // B, n % B
            bl = 2 * W // NS - A
            for st, ln, p in ((s * A, A, 0), (NS * A + s * bl, bl, 1)):
                parts = []
                if st < W:
                    parts.append((0, st, min(ln, W - st)))
                if st + ln > W:
                    s2 = max(st, W)
                    parts.append((1, s2 - W, st + ln - s2))
                for which, r, l in parts:
                    src, dst = ((k_hbm, kb), (v_hbm, vb))[which]
                    cp(src.at[b, h, pl.ds(row0 + r, l)], dst.at[slot, pl.ds(r, l)],
                       sem_kv.at[which, slot], p)

        def ffn_step(i):
            r = ds(i, FR)
            cp(w1t_hbm.at[r], w1t_v.at[r], sem_w.at[3], 0)
            cp(w2_hbm.at[r], w2_v.at[r], sem_f.at[(i * FR) // 128], 1)

        wmod_step(0, None)
        cp(c_hbm, c_v, sem_s.at[0], 0)
        cp(x_hbm, x_v, sem_s.at[1], 0)
        cp(b1_hbm, b1_v, sem_s.at[2], 0)
        cp(b2_hbm, b2_v, sem_s.at[3], 0)
        lax.fori_loop(1, D // 32, wmod_step, None)
        lax.fori_loop(0, D // 32, wq_step, None)

        wait(c_v, sem_s.at[0])
        wait(wmod_v, sem_w.at[0])
        cf = c_v[...].astype(F32)
        sc = (cf / (1.0 + jnp.exp(-cf))).astype(BF16)
        h_v[...] = sc

        def mod_body(j, _):
            wo_step(2 * j)
            wo_step(2 * j + 1)
            mod_v[j] = _dot(h_v[...], wmod_v[:, ds(j, 128)])

        lax.fori_loop(0, 6 * D // 128, mod_body, None)
        for i in range(60, 64):
            wo_step(i)

        def mod(i):
            n = D // 128
            return jnp.concatenate([mod_v[i * n + j] for j in range(n)], axis=1)

        wait(x_v, sem_s.at[1])
        h_v[...] = (_layernorm(x_v[...].astype(F32)) * (1.0 + mod(1)) + mod(0)).astype(BF16)
        acc_v[...] = jnp.zeros(acc_v.shape, F32)
        oh_v[...] = jnp.zeros(oh_v.shape, F32)

        def kv_all(n, _):
            for s in range(NS):
                kv_step(n, n, s)

        lax.fori_loop(0, DEPTH, kv_all, None)
        wait(wq_v, sem_w.at[1])
        wait(wo_v, sem_w.at[2])

        NC = W // CT

        def attn(n, slot, issue, nsteps):
            h, b = n // B, n % B

            @pl.when(b == 0)
            def _():
                q_v[...] = _dot(h_v[...], wq_v[:, ds(h, DH)]).astype(BF16)

            done = [0]

            def issue_upto(k):
                t = -(-k * nsteps // (2 * NC))
                while done[0] < t:
                    issue(done[0])
                    done[0] += 1

            q = q_v[...]
            wait(kb.at[slot], sem_kv.at[0, slot])
            ss = []
            for j in range(NC):
                issue_upto(j + 1)
                ss.append(_dot_t(q, kb[slot, pl.ds(j * CT, CT)]) * DH ** -0.5)
            m = functools.reduce(jnp.maximum, ss)
            m = jnp.max(m, axis=-1, keepdims=True)
            ps = [jnp.exp(s - m) for s in ss]
            l = jnp.sum(functools.reduce(jnp.add, ps), axis=-1, keepdims=True)
            wait(vb.at[slot], sem_kv.at[1, slot])
            o = None
            for j in range(NC):
                issue_upto(NC + j + 1)
                t = _dot(ps[j].astype(BF16), vb[slot, pl.ds(j * CT, CT)])
                o = t if o is None else o + t
            o = o / l
            rows = lax.broadcasted_iota(jnp.int32, o.shape, 0)
            oh = jnp.where(rows == b, o, oh_v[...])
            oh_v[...] = oh

            @pl.when(b == B - 1)
            def _():
                acc_v[...] += _dot(oh.astype(BF16), wo_v[ds(h, DH)])

        def nxt(slot):
            return jnp.where(slot == R - 1, 0, slot + 1)

        def body1(n, slot):
            prev = jnp.where(slot == 0, R - 1, slot - 1)
            attn(n, slot, lambda s: kv_step(n + DEPTH, prev, s), NS)
            return nxt(slot)

        FS = F // FR // DEPTH
        assert FS * FR * DEPTH == F

        def body2(n, slot):
            attn(n, slot, lambda s: ffn_step((n - (N - DEPTH)) * FS + s), FS)
            return nxt(slot)

        slot = lax.fori_loop(0, N - DEPTH, body1, jnp.int32(0))
        lax.fori_loop(N - DEPTH, N, body2, slot)

        x1 = x_v[...].astype(F32) + mod(2) * acc_v[...]
        h2 = (_layernorm(x1) * (1.0 + mod(4)) + mod(3)).astype(BF16)
        wait(b1_v, sem_s.at[2])
        wait(b2_v, sem_s.at[3])
        wait(w1t_v, sem_w.at[3])
        b1 = b1_v[...].astype(F32).reshape(1, F)
        g = _gelu(_dot_t(h2, w1t_v[...]) + b1).astype(BF16)
        y = b2_v[...].astype(F32).reshape(1, D)
        for j in range(pl.cdiv(F, 128)):
            n = min(128, F - j * 128)
            wait(w2_v.at[pl.ds(j * 128, n)], sem_f.at[j])
            y = y + _dot(g[:, j * 128:j * 128 + n], w2_v[pl.ds(j * 128, n)])
        o_ref[...] = (x1 + mod(5) * y).astype(o_ref.dtype)

    def fn(A_x, A_k_cache, A_v_cache, A_wq, A_wo, B_x, B_w1, B_b1, B_w2, B_b2, c, w_mod):
        B, S, D = A_x.shape
        _, H, SK, DH = A_k_cache.shape
        W = min(4096, max(256, SK // 4))
        F = B_w2.shape[0]
        R = DEPTH + 1
        V = pltpu.VMEM
        out = pl.pallas_call(
            kern,
            out_shape=jax.ShapeDtypeStruct((B, D), A_x.dtype),
            in_specs=[pl.BlockSpec(memory_space=pltpu.HBM)] * 11,
            out_specs=pl.BlockSpec(memory_space=pltpu.VMEM),
            scratch_shapes=[
                V((B, D), BF16), V((B, D), BF16), V((F,), BF16), V((D,), BF16),
                V((D, 6 * D), BF16), V((D, H * DH), BF16), V((H * DH, D), BF16),
                V((F, D), BF16), V((F, D), BF16),
                V((R, W, DH), BF16), V((R, W, DH), BF16),
                V((6 * D // 128, B, 128), F32), V((B, D), BF16), V((B, DH), BF16),
                V((B, DH), F32), V((B, D), F32),
                pltpu.SemaphoreType.DMA((4,)), pltpu.SemaphoreType.DMA((4,)),
                pltpu.SemaphoreType.DMA((2, R)), pltpu.SemaphoreType.DMA((pl.cdiv(F, 128),)),
            ],
            compiler_params=pltpu.CompilerParams(vmem_limit_bytes=100 * 2**20),
            name="adaln_decode",
        )(A_x.reshape(B, D), c, B_b1, B_b2, w_mod, A_wq, A_wo, B_w1.T, B_w2,
          A_k_cache, A_v_cache)
        return out.reshape(B, S, D)

    return fn


_fn = make()


@jax.jit
def pallas_adaLN_cond__sliding_block_cached__dense_activation_gelu__decode_kernel(
    A_x, A_k_cache, A_v_cache, A_wq, A_wo, B_x, B_w1, B_b1, B_w2, B_b2, c, w_mod):
    return _fn(A_x, A_k_cache, A_v_cache, A_wq, A_wo, B_x, B_w1, B_b1, B_w2, B_b2, c, w_mod)
```

```python
import functools
import math

import jax
import jax.numpy as jnp
from jax import lax
import jax.experimental.pallas as pl
import jax.experimental.pallas.tpu as pltpu

F32 = jnp.float32
BF16 = jnp.bfloat16

HEADS = 4
KV_ROWS = 32
SLOTS = 3
SEGS = 8
FF_ROWS = 32
FF_CHUNKS = (0, 1024, 1536, 1728)


def _dot(a, b):
    return lax.dot_general(a, b, (((1,), (0,)), ((), ())), preferred_element_type=F32)


def _dot_t(a, b):
    return lax.dot_general(a, b, (((1,), (1,)), ((), ())), preferred_element_type=F32)


def _layernorm(x):
    d = x - jnp.mean(x, axis=-1, keepdims=True)
    v = jnp.mean(d * d, axis=-1, keepdims=True)
    return d / jnp.sqrt(v + 1e-05)


def _gelu(x):
    k = math.sqrt(2.0 / math.pi)
    return 0.5 * x * (1.0 + jnp.tanh(k * (x + 0.044715 * (x * x * x))))


def _start(src, dst, sem, priority):
    pltpu.make_async_copy(src, dst, sem).start(priority=priority)


def _wait(buf, sem):
    pltpu.make_async_copy(buf, buf, sem).wait()


def _ds(i, n):
    return pl.ds(pl.multiple_of(i * n, n), n)


def _main(x_hbm, c_hbm, b1_hbm, b2_hbm, wmod_hbm, wq_hbm, wo_hbm, w1t_hbm, w2_hbm,
          k_hbm, v_hbm, o_hbm,
          x_v, c_v, b1_v, b2_v, wmod_v, wq_v, wo_v, w1t_v, w2_v, k_v, v_v,
          mod_v, h_v, q_v, oh_v, acc_v, o_v, sem_o,
          sem_s, sem_w, sem_kv, sem_1, sem_2):
    B, D = x_hbm.shape
    _, H, SK, DH = k_hbm.shape
    W = k_v.shape[2]
    F = w2_hbm.shape[0]
    kv_steps = W // KV_ROWS

    def seg_step(src, dst, sem, i, cols):
        for p in range(2):
            idx = (pl.ds(p * SEGS // 2, SEGS // 2), _ds(i, 8), cols)
            _start(src.at[idx], dst.at[idx], sem, p)

    def wmod_rows(i, _):
        for j in range(6):
            seg_step(wmod_hbm, wmod_v, sem_w.at[0], i, pl.ds(j * D, D))

    def wq_rows(i, _):
        for j in range(H * DH // 512):
            seg_step(wq_hbm, wq_v, sem_w.at[1], i, pl.ds(j * 512, 512))

    def wo_step(i):
        seg_step(wo_hbm, wo_v, sem_w.at[2], i, slice(None))

    def kv_step(g, s):
        b, h, slot = g // (H // HEADS), g % (H // HEADS) * HEADS, g % SLOTS
        rows = pl.ds(pl.multiple_of(SK - W + s * KV_ROWS, KV_ROWS), KV_ROWS)
        for p, (src, dst) in enumerate(((k_hbm, k_v), (v_hbm, v_v))):
            _start(src.at[b, pl.ds(h, HEADS), rows], dst.at[slot, :, _ds(s, KV_ROWS)],
                   sem_kv.at[p, slot], p)

    def ffn_step(i):
        rows = _ds(i, FF_ROWS)
        chunk = sum((i * FF_ROWS >= t).astype(jnp.int32) for t in FF_CHUNKS[1:-1])
        _start(w1t_hbm.at[rows], w1t_v.at[rows], sem_1.at[chunk], 0)
        _start(w2_hbm.at[rows], w2_v.at[rows], sem_2.at[chunk], 1)

    wmod_rows(0, None)
    _start(c_hbm, c_v, sem_s.at[0], 0)
    _start(x_hbm, x_v, sem_s.at[1], 0)
    _start(b1_hbm, b1_v, sem_s.at[2], 0)
    _start(b2_hbm, b2_v, sem_s.at[3], 0)
    lax.fori_loop(1, D // SEGS // 8, wmod_rows, None)
    lax.fori_loop(0, D // SEGS // 8, wq_rows, None)

    _wait(c_v, sem_s.at[0])
    _wait(wmod_v, sem_w.at[0])
    cf = c_v[...].astype(F32)
    h_v[...] = (cf / (1.0 + jnp.exp(-cf))).astype(BF16)

    def mod_tile(j, _):
        wo_step(2 * j)
        wo_step(2 * j + 1)
        mod_v[j] = _dot(h_v[...], wmod_v[:, :, _ds(j, 128)].reshape(D, 128))

    lax.fori_loop(0, 6 * D // 128, mod_tile, None)
    for i in range(2 * 6 * D // 128, H * DH // SEGS // 8):
        wo_step(jnp.int32(i))

    def mod(i):
        n = D // 128
        return jnp.concatenate([mod_v[i * n + j] for j in range(n)], axis=1)

    _wait(x_v, sem_s.at[1])
    h_v[...] = (_layernorm(x_v[...].astype(F32)) * (1.0 + mod(1)) + mod(0)).astype(BF16)
    acc_v[...] = jnp.zeros(acc_v.shape, F32)
    oh_v[...] = jnp.zeros(oh_v.shape, F32)

    def kv_fill(i, _):
        for s in range(4):
            kv_step(i // (kv_steps // 4), i % (kv_steps // 4) * 4 + s)

    lax.fori_loop(0, (SLOTS - 1) * kv_steps // 4, kv_fill, None)
    _wait(wq_v, sem_w.at[1])
    _wait(wo_v, sem_w.at[2])

    def attend(n, issue, nsteps):
        b, h, slot, hi = n // H, n % H, n // HEADS % SLOTS, n % HEADS

        @pl.when(b == 0)
        def _():
            q_v[h] = _dot(h_v[...], wq_v[:, :, _ds(h, DH)].reshape(D, DH)).astype(BF16)

        @pl.when(hi == 0)
        def _():
            _wait(k_v.at[slot], sem_kv.at[0, slot])
            _wait(v_v.at[slot], sem_kv.at[1, slot])

        nt = W // 128

        def issue_for_tile(t):
            for s in range(pl.cdiv(t * nsteps, 2 * nt), pl.cdiv((t + 1) * nsteps, 2 * nt)):
                issue(s)

        q = q_v[h]
        ss = []
        for j in range(nt):
            issue_for_tile(j)
            ss.append(_dot_t(q, k_v[slot, hi, pl.ds(j * 128, 128)]) * DH ** -0.5)
        m = jnp.max(functools.reduce(jnp.maximum, ss), axis=-1, keepdims=True)
        ps = [jnp.exp(s - m) for s in ss]
        denom = jnp.sum(functools.reduce(jnp.add, ps), axis=-1, keepdims=True)
        o = None
        for j in range(nt):
            issue_for_tile(nt + j)
            t = _dot(ps[j].astype(BF16), v_v[slot, hi, pl.ds(j * 128, 128)])
            o = t if o is None else o + t
        row = lax.broadcasted_iota(jnp.int32, o.shape, 0)
        oh = jnp.where(row == b, o / denom, oh_v[h])
        oh_v[h] = oh

        @pl.when(b == B - 1)
        def _():
            acc_v[...] += _dot(oh.astype(BF16), wo_v[h // (H // SEGS), _ds(h % (H // SEGS), DH)])

    n1 = B * H - (SLOTS - 1) * HEADS
    ks = kv_steps // HEADS
    fs, f0 = divmod(F // FF_ROWS, HEADS)
    lax.fori_loop(0, n1, lambda n, _: attend(
        n, lambda s: kv_step(n // HEADS + SLOTS - 1, n % HEADS * ks + s), ks), None)
    for i in range(f0):
        ffn_step(jnp.int32(i))
    lax.fori_loop(n1, n1 + HEADS, lambda n, _: attend(
        n, lambda s: ffn_step(f0 + (n - n1) * fs + s), fs), None)
    lax.fori_loop(n1 + HEADS, B * H, lambda n, _: attend(n, None, 0), None)

    x1 = x_v[...].astype(F32) + mod(2) * acc_v[...]
    h2 = (_layernorm(x1) * (1.0 + mod(4)) + mod(3)).astype(BF16)
    _wait(b1_v, sem_s.at[2])
    _wait(b2_v, sem_s.at[3])
    b1 = b1_v[...].astype(F32).reshape(1, F)
    chunks = list(zip(FF_CHUNKS[:-1], FF_CHUNKS[1:]))
    gs = []
    for j, (a, e) in enumerate(chunks):
        _wait(w1t_v.at[a:e], sem_1.at[j])
        gs.append(_gelu(_dot_t(h2, w1t_v[a:e]) + b1[:, a:e]).astype(BF16))
    y = b2_v[...].astype(F32).reshape(1, D)
    for j, (a, e) in enumerate(chunks):
        _wait(w2_v.at[a:e], sem_2.at[j])
        y = y + _dot(gs[j], w2_v[a:e])
    o_v[...] = (x1 + mod(5) * y).astype(o_v.dtype)
    _start(o_v, o_hbm, sem_o, 0)


def _kernel(*refs):
    o_hbm, o_v, sem_o = refs[11], refs[-2], refs[-1]
    dma = pltpu.SemaphoreType.DMA
    nc = len(FF_CHUNKS) - 1
    pl.run_scoped(functools.partial(_main, *refs),
                  dma((4,)), dma((3,)), dma((2, SLOTS)), dma((nc,)), dma((nc,)))
    pltpu.make_async_copy(o_v, o_hbm, sem_o).wait()


@jax.jit
def pallas_adaLN_cond__sliding_block_cached__dense_activation_gelu__decode_kernel(
    A_x: jax.Array,
    A_k_cache: jax.Array,
    A_v_cache: jax.Array,
    A_wq: jax.Array,
    A_wo: jax.Array,
    B_x: jax.Array,
    B_w1: jax.Array,
    B_b1: jax.Array,
    B_w2: jax.Array,
    B_b2: jax.Array,
    c: jax.Array,
    w_mod: jax.Array,
):
    del B_x
    B, S, D = A_x.shape
    _, H, SK, DH = A_k_cache.shape
    W = min(4096, max(256, SK // 4))
    F = B_w2.shape[0]
    assert S == 1 and F == FF_CHUNKS[-1]
    vmem = pltpu.VMEM
    w_mod, A_wq, A_wo = (w.reshape(SEGS, w.shape[0] // SEGS, w.shape[1])
                         for w in (w_mod, A_wq, A_wo))
    out = pl.pallas_call(
        _kernel,
        out_shape=jax.ShapeDtypeStruct((B, D), A_x.dtype),
        in_specs=[pl.BlockSpec(memory_space=pltpu.HBM)] * 11,
        out_specs=pl.BlockSpec(memory_space=pltpu.HBM),
        scratch_shapes=[
            vmem((B, D), BF16), vmem((B, D), BF16), vmem((F,), BF16), vmem((D,), BF16),
            vmem(w_mod.shape, BF16), vmem(A_wq.shape, BF16), vmem(A_wo.shape, BF16),
            vmem((F, D), BF16), vmem((F, D), BF16),
            vmem((SLOTS, HEADS, W, DH), BF16), vmem((SLOTS, HEADS, W, DH), BF16),
            vmem((6 * D // 128, B, 128), F32), vmem((B, D), BF16),
            vmem((H, B, DH), BF16), vmem((H, B, DH), F32), vmem((B, D), F32),
            vmem((B, D), BF16), pltpu.SemaphoreType.DMA(()),
        ],
        compiler_params=pltpu.CompilerParams(
            vmem_limit_bytes=64 * 2**20, disable_bounds_checks=True),
        name="adaln_decode",
    )(A_x.reshape(B, D), c, B_b1, B_b2, w_mod, A_wq, A_wo, B_w1.T, B_w2,
      A_k_cache, A_v_cache)
    return out.reshape(B, S, D)
```
